```python
import jax
import jax.numpy as jnp

def _softmax(x, axis=-1):
    return jax.nn.softmax(x, axis=axis)
def _gelu(x):
    return jax.nn.gelu(x, approximate=True)
def _silu(x):
    return jax.nn.silu(x)
def _sigmoid(x):
    return jax.nn.sigmoid(x)
def _layernorm(x, axis=-1, eps=1e-5):
    m = jnp.mean(x, axis=axis, keepdims=True)
    v = jnp.var(x, axis=axis, keepdims=True)
    return (x - m) / jnp.sqrt(v + eps)
def _scatter_add(tgt, idx, src, axis=0):
    return tgt.at[idx].add(src)
def _segment_sum(src, seg, n):
    return jax.ops.segment_sum(src, seg, n)
class _Rng:
    def __init__(self, key):
        self._k = key
    def _next(self):
        self._k, sub = jax.random.split(self._k)
        return sub
    def normal(self, shape):
        return jax.random.normal(self._next(), shape, dtype=jnp.bfloat16)
    def randint(self, lo, hi, shape):
        return jax.random.randint(self._next(), shape, lo, hi, dtype=jnp.int32)
    def uniform(self, shape, lo=0.0, hi=1.0):
        return jax.random.uniform(self._next(), shape, jnp.bfloat16, lo, hi)
    def permutation(self, n):
        return jax.random.permutation(self._next(), n)


kernel_name = 'interleave_layers__softmax_full_mha__ssm_conv_h3__prompt'

def setup_inputs():
    _rng = _Rng(jax.random.key(int.from_bytes(__import__("os").urandom(4), "little")))
    _w = (lambda a: (lambda t: t.astype(jnp.bfloat16) if jnp.issubdtype(t.dtype, jnp.floating) else t)(jnp.asarray(a)))
    def _A_setup():
        B, S, D = 1, 2048, 1024
        return {
            "x": _w((lambda *s: _rng.normal(s) * 0.05)(B, S, D)),
            "wqkv": _w((lambda *s: _rng.normal(s) * 0.05)(D, 3 * D)),
            "wo": _w((lambda *s: _rng.normal(s) * 0.05)(D, D)),
        }
    _A_in = _A_setup()

    def _B_setup():
        B, S, D = 1, 2048, 1024
        ks = 4
        return {
            "q": _w((lambda *s: _rng.normal(s) * 0.05)(B, S, D)),
            "k": _w((lambda *s: _rng.normal(s) * 0.05)(B, S, D)),
            "v": _w((lambda *s: _rng.normal(s) * 0.05)(B, S, D)),
            "shift_k": _w((lambda *s: _rng.normal(s) * 0.05)(D, ks) * 0.5),
            "ssm_k": _w((lambda *s: _rng.normal(s) * 0.05)(D, S) * (1.0 / S ** 0.5)),
            "ssm_D": _w((lambda *s: _rng.normal(s) * 0.05)(D)),
        }
    _B_in = _B_setup()

    return {
        "A_x": _A_in["x"],
        "A_wqkv": _A_in["wqkv"],
        "A_wo": _A_in["wo"],
        "B_q": _B_in["q"],
        "B_k": _B_in["k"],
        "B_v": _B_in["v"],
        "B_shift_k": _B_in["shift_k"],
        "B_ssm_k": _B_in["ssm_k"],
        "B_ssm_D": _B_in["ssm_D"],
    }

def reference(A_x, A_wqkv, A_wo, B_q, B_k, B_v, B_shift_k, B_ssm_k, B_ssm_D):
    def _A_ref(x, wqkv, wo):
        B, S, D = x.shape
        H = 32; Dh = D // H
        qkv = (lambda x, *d: x.transpose(*d))((x @ wqkv).reshape(B, S, 3, H, Dh), 2, 0, 3, 1, 4)
        q, k, v = qkv[0], qkv[1], qkv[2]
        scale = Dh ** -0.5
        scores = jnp.einsum("bhqd,bhkd->bhqk", q, k) * scale
        p = _softmax(scores, axis=-1)
        o = jnp.einsum("bhqk,bhkd->bhqd", p, v)
        return (lambda x, *d: x.transpose(*d))(o, 0, 2, 1, 3).reshape(B, S, D) @ wo

    def _B_ref(q, k, v, shift_k, ssm_k, ssm_D):
        B, S, D = q.shape
        ks = shift_k.shape[-1]
        k_pad = jnp.pad(k, ((0, 0), (ks - 1, 0), (0, 0)))
        k_shift = jnp.zeros_like(k)
        for t in range(ks):
            k_shift = k_shift + k_pad[:, t:t + S, :] * shift_k[:, ks - 1 - t][None, None, :]
        kv = k_shift * v
        L = 2 * S
        kv_pad = jnp.pad(kv, ((0, 0), (0, S), (0, 0)))
        kf_pad = jnp.pad(ssm_k, ((0, 0), (0, S)))
        kv_f = (lambda x, axes=(-2,-1): jnp.fft.rfft2(x.astype(jnp.float32), axes=axes))(kv_pad[:, None, :, :], axes=(1, 2))
        kf_f = (lambda x, axes=(-2,-1): jnp.fft.rfft2(x.astype(jnp.float32), axes=axes))(kf_pad[:, None, :], axes=(1, 2))
        kf_f = (lambda x, *d: x.transpose(*d))(kf_f, 1, 2, 0)
        y_f = kv_f * kf_f[None, :, :, :]
        y = (lambda x, s, axes=(-2,-1): jnp.fft.irfft2(x, s=s, axes=axes).astype(jnp.bfloat16))(y_f, (1, L), axes=(1, 2))[:, 0, :S, :]
        y = y + kv * ssm_D[None, None, :]
        return q * y

    x = A_x
    x = x + _A_ref(_layernorm(x, axis=-1), A_wqkv, A_wo)
    x = x + _B_ref(_layernorm(x, axis=-1), B_k, B_v, B_shift_k, B_ssm_k, B_ssm_D)
    x = x + _A_ref(_layernorm(x, axis=-1), A_wqkv, A_wo)
    x = x + _B_ref(_layernorm(x, axis=-1), B_k, B_v, B_shift_k, B_ssm_k, B_ssm_D)
    return x
```

```python
import math

import jax
import jax.numpy as jnp
import numpy as np
from jax import lax
from jax.experimental import pallas as pl
from jax.experimental.pallas import tpu as pltpu

S, D, H, DH = 2048, 1024, 32, 32
TQ = 256
KC = 128
TT = 256
L = 128
NL = S // L
CT = 256
NQ = S // TQ
LNQ = NQ.bit_length() - 1
F32 = jnp.float32
BF16 = jnp.bfloat16
NT = (((1,), (1,)), ((), ()))
TN = (((0,), (0,)), ((), ()))


def _dft_consts():
    f = np.arange(L, dtype=np.float64)
    th = np.pi * (2 * f + 1) / (2 * L)
    t = np.arange(L, dtype=np.float64)
    fwd = np.concatenate([np.cos(th[:, None] * t[None]), -np.sin(th[:, None] * t[None])], 0)
    t2 = np.arange(2 * L, dtype=np.float64)
    inv = np.concatenate([np.cos(t2[:, None] * th[None]), -np.sin(t2[:, None] * th[None])], 1) / L
    return fwd.astype(np.float32), inv.astype(np.float32)


def _ln(x):
    m = jnp.mean(x, axis=-1, keepdims=True)
    xc = x - m
    v = jnp.mean(xc * xc, axis=-1, keepdims=True)
    return xc * lax.rsqrt(v + 1e-5)


def _kernel(x_hbm, w_hbm, wo_hbm, k_hbm, v_hbm, sh_ref, sk_hbm, sd_ref, fw_ref, gi_ref,
            out_hbm,
            xin, xres, w, wo, wqT, wvT, qT, kk, vT, oT, sa, sb, y, kin, vin, skv,
            kpad, uf, kf, yf, sems):
    cps = [pltpu.make_async_copy(a, b, sems.at[i]) for i, (a, b) in enumerate(
        [(x_hbm, xin), (w_hbm, w), (k_hbm, kin), (v_hbm, vin), (sk_hbm, skv), (wo_hbm, wo)])]
    for c in cps:
        c.start()
    qscale = (DH ** -0.5) * math.log2(math.e)

    def proj(r0, xt):
        xn = _ln(xt).astype(BF16)
        kk[pl.ds(r0, TT), :] = jnp.dot(xn, w[:, D:2 * D], preferred_element_type=F32).astype(BF16)
        qT[:, pl.ds(r0, TT)] = (lax.dot_general(wqT[...], xn, NT, preferred_element_type=F32)
                                * qscale).astype(BF16)
        vT[:, pl.ds(r0, TT)] = lax.dot_general(wvT[...], xn, NT, preferred_element_type=F32).astype(BF16)

    cps[1].wait()

    def tr_body(i, c):
        c0 = pl.multiple_of(i * 128, 128)
        wqT[pl.ds(c0, 128), :] = w[:, pl.ds(c0, 128)].T
        wvT[pl.ds(c0, 128), :] = w[:, pl.ds(pl.multiple_of(2 * D + c0, 128), 128)].T
        return c
    lax.fori_loop(0, D // 128, tr_body, 0)
    cps[0].wait()

    def proj1(t, c):
        r0 = pl.multiple_of(t * TT, TT)
        xt = xin[pl.ds(r0, TT), :].astype(F32)
        xres[pl.ds(r0, TT), :] = xt
        proj(r0, xt)
        return c
    lax.fori_loop(0, S // TT, proj1, 0)

    cps[2].wait()
    cps[3].wait()
    cps[4].wait()
    kpad[pl.ds(0, 8), :] = jnp.zeros((8, CT), F32)

    def ssm_tile(ct, c):
        c0 = pl.multiple_of(ct * CT, CT)
        cs = pl.ds(c0, CT)
        sh = sh_ref[:, cs]
        dd = sd_ref[:, cs].astype(F32)
        kpad[pl.ds(8, S), :] = kin[:, cs].astype(F32)
        fw = fw_ref[...]

        def fwd(j, c2):
            r0 = pl.multiple_of(j * L, L)
            kx = kpad[pl.ds(r0, L + 8), :]
            ks = kx[8:] * sh[0:1]
            for d in range(1, 4):
                ks = ks + kx[8 - d:8 - d + L] * sh[d:d + 1]
            kv = ks * vin[pl.ds(r0, L), cs].astype(F32)
            y[pl.ds(r0, L), cs] = kv * dd
            uf[j] = jnp.dot(fw, kv.astype(BF16), preferred_element_type=F32)
            kf[j] = lax.dot_general(fw, skv[cs, pl.ds(r0, L)], NT, preferred_element_type=F32)
            return c2
        lax.fori_loop(0, NL, fwd, 0)

        def prod(fb, c2):
            f0 = pl.multiple_of(fb * 16, 16)
            for cc in range(CT // 128):
                ls = slice(cc * 128, (cc + 1) * 128)
                res = []
                for hf in range(2):
                    fr = pl.ds(pl.multiple_of(f0 + hf * 8, 8), 8)
                    fi = pl.ds(pl.multiple_of(f0 + hf * 8 + L, 8), 8)
                    ur = [uf[j, fr, ls] for j in range(NL)]
                    ui = [uf[j, fi, ls] for j in range(NL)]
                    rr = []
                    for i in range(NL):
                        ar = ai = None
                        for j in range(i + 1):
                            kr = kf[i - j, fr, ls]
                            ki = kf[i - j, fi, ls]
                            pr = kr * ur[j] - ki * ui[j]
                            pi = kr * ui[j] + ki * ur[j]
                            ar = pr if ar is None else ar + pr
                            ai = pi if ai is None else ai + pi
                        rr.append((ar, ai))
                    res.append(rr)
                for i in range(NL):
                    yf[i, pl.ds(f0, 16), ls] = jnp.concatenate(
                        [res[0][i][0], res[1][i][0]], 0).astype(BF16)
                    yf[i, pl.ds(pl.multiple_of(f0 + L, 16), 16), ls] = jnp.concatenate(
                        [res[0][i][1], res[1][i][1]], 0).astype(BF16)
            return c2
        lax.fori_loop(0, L // 16, prod, 0)

        gi = gi_ref[...]

        def inv(i, hi):
            r0 = pl.multiple_of(i * L, L)
            r = jnp.dot(gi, yf[i], preferred_element_type=F32)
            y[pl.ds(r0, L), cs] = y[pl.ds(r0, L), cs] + (r[:L] + hi)
            return r[L:]
        lax.fori_loop(0, NL, inv, jnp.zeros((L, CT), F32))
        return c
    lax.fori_loop(0, D // CT, ssm_tile, 0)
    cps[5].wait()

    row = lax.broadcasted_iota(jnp.int32, (128, TQ), 0)
    nit = H * NQ

    def qk_setup(it):
        h = it >> LNQ
        qt = it & (NQ - 1)
        g = h >> 2
        hh = h & 3
        q = qT[pl.ds(pl.multiple_of(g * 128, 128), 128), pl.ds(pl.multiple_of(qt * TQ, TQ), TQ)]
        qm = jnp.where((row >> 5) == hh, q.astype(F32), 0.0).astype(BF16)
        return g, qm

    def qk_chunk(g, qm, kc, sref):
        kt = kk[pl.ds(kc * KC, KC), pl.ds(pl.multiple_of(g * 128, 128), 128)]
        s = jnp.dot(kt, qm, preferred_element_type=F32)
        sref[pl.ds(kc * KC, KC), :] = s
        return jnp.max(s.reshape(KC // 8, 8, TQ), axis=0)

    def step(it, cur, nxt, mprev8):
        mprev = jnp.max(mprev8, axis=0, keepdims=True)
        h = it >> LNQ
        qt = it & (NQ - 1)
        g, qm = qk_setup(jnp.minimum(it + 1, nit - 1))
        m = acc = l = None
        for kc in range(S // KC):
            mc = qk_chunk(g, qm, kc, nxt)
            m = mc if m is None else jnp.maximum(m, mc)
            p = jnp.exp2(cur[pl.ds(kc * KC, KC), :] - mprev)
            lc = jnp.sum(p.reshape(KC // 8, 8, TQ), axis=0)
            l = lc if l is None else l + lc
            vt = vT[pl.ds(pl.multiple_of(h * DH, DH), DH), pl.ds(kc * KC, KC)]
            a = jnp.dot(vt, p.astype(BF16), preferred_element_type=F32)
            acc = a if acc is None else acc + a
        o = acc * (1.0 / jnp.sum(l, axis=0, keepdims=True))
        oT[pl.ds(pl.multiple_of(h * DH, DH), DH), pl.ds(pl.multiple_of(qt * TQ, TQ), TQ)] = o.astype(BF16)
        return m

    def attention():
        g, qm = qk_setup(0)
        m = None
        for kc in range(S // KC):
            mc = qk_chunk(g, qm, kc, sa)
            m = mc if m is None else jnp.maximum(m, mc)

        def body(i2, m):
            m = step(2 * i2, sa, sb, m)
            return step(2 * i2 + 1, sb, sa, m)
        lax.fori_loop(0, nit // 2, body, m)

    def post(r0):
        rs = pl.ds(r0, TT)
        x1 = xres[rs, :] + lax.dot_general(oT[:, rs], wo[...], TN, preferred_element_type=F32)
        return x1 + _ln(x1) * y[rs, :]

    def layer(li, c):
        attention()

        @pl.when(li == 0)
        def _():
            def mid(t, c2):
                r0 = pl.multiple_of(t * TT, TT)
                x2 = post(r0)
                xres[pl.ds(r0, TT), :] = x2
                proj(r0, x2)
                return c2
            lax.fori_loop(0, S // TT, mid, 0)
        return c
    lax.fori_loop(0, 2, layer, 0)

    def out_copy(t):
        r0 = pl.multiple_of(t * TT, TT)
        return pltpu.make_async_copy(xin.at[pl.ds(r0, TT), :], out_hbm.at[pl.ds(r0, TT), :], sems.at[6])

    def fin(t, c):
        r0 = pl.multiple_of(t * TT, TT)
        xin[pl.ds(r0, TT), :] = post(r0).astype(BF16)
        out_copy(t).start()
        return c
    lax.fori_loop(0, S // TT, fin, 0)
    pltpu.make_async_copy(xin, out_hbm, sems.at[6]).wait()


@jax.jit
def pallas_interleave_layers__softmax_full_mha__ssm_conv_h3__prompt_kernel(
    A_x, A_wqkv, A_wo, B_q, B_k, B_v, B_shift_k, B_ssm_k, B_ssm_D,
):
    fwd, inv = _dft_consts()
    any_spec = pl.BlockSpec(memory_space=pl.ANY)
    vmem_spec = pl.BlockSpec(memory_space=pltpu.VMEM)
    vm = pltpu.VMEM
    out = pl.pallas_call(
        _kernel,
        out_shape=jax.ShapeDtypeStruct((S, D), BF16),
        in_specs=[any_spec] * 5 + [vmem_spec, any_spec, vmem_spec, vmem_spec, vmem_spec],
        out_specs=any_spec,
        scratch_shapes=[
            vm((S, D), BF16), vm((S, D), F32), vm((D, 3 * D), BF16), vm((D, D), BF16),
            vm((D, D), BF16), vm((D, D), BF16),
            vm((D, S), BF16), vm((S, D), BF16), vm((D, S), BF16), vm((D, S), BF16),
            vm((S, TQ), F32), vm((S, TQ), F32), vm((S, D), F32),
            vm((S, D), BF16), vm((S, D), BF16), vm((D, S), BF16),
            vm((S + 8, CT), F32), vm((NL, 2 * L, CT), F32), vm((NL, 2 * L, CT), F32),
            vm((NL, 2 * L, CT), BF16),
            pltpu.SemaphoreType.DMA((7,)),
        ],
        compiler_params=pltpu.CompilerParams(vmem_limit_bytes=120 * 1024 * 1024),
    )(A_x.reshape(S, D), A_wqkv, A_wo, B_k.reshape(S, D), B_v.reshape(S, D),
      B_shift_k.T.astype(F32), B_ssm_k, B_ssm_D.reshape(1, D),
      jnp.asarray(fwd, BF16), jnp.asarray(inv, BF16))
    return out.reshape(A_x.shape)
```

```python
import math

import jax
import jax.numpy as jnp
import numpy as np
from jax import lax
from jax.experimental import pallas as pl
from jax.experimental.pallas import tpu as pltpu

S, D, H, DH = 2048, 1024, 32, 32
TQ = 256
KC = 128
TT = 256
L = 128
NL = S // L
LEAD = 4
UN = 8
NP = 4
NQ = S // TQ
LNQ = NQ.bit_length() - 1
F32 = jnp.float32
BF16 = jnp.bfloat16
NT = (((1,), (1,)), ((), ()))
TN = (((0,), (0,)), ((), ()))


def _dft_consts():
    f = np.arange(L, dtype=np.float64)
    th = np.pi * (2 * f + 1) / (2 * L)
    t = np.arange(L, dtype=np.float64)
    fwd = np.concatenate([np.cos(th[:, None] * t[None]), -np.sin(th[:, None] * t[None])], 0)
    t2 = np.arange(2 * L, dtype=np.float64)
    inv = np.concatenate([np.cos(t2[:, None] * th[None]), -np.sin(t2[:, None] * th[None])], 1) / L
    return fwd.astype(np.float32), inv.astype(np.float32)


def _ln(x):
    m = jnp.mean(x, axis=-1, keepdims=True)
    xc = x - m
    v = jnp.mean(xc * xc, axis=-1, keepdims=True)
    return xc * lax.rsqrt(v + 1e-5)


def _kernel(x_hbm, w_hbm, wo_hbm, k_hbm, v_hbm, sh_ref, sk_hbm, sd_ref, fw_ref, gi_ref,
            out_hbm,
            xin, xres, w, wo, wqT, wvT, qT, kk, vT, oT, sa, sb, y, kin, vin, skv,
            uf, kf, sems):
    cps = [pltpu.make_async_copy(a, b, sems.at[i]) for i, (a, b) in enumerate(
        [(x_hbm, xin), (w_hbm, w), (wo_hbm, wo)])]
    pieces = []
    for q in range(NP):
        ts = pl.ds(q * (S // NP), S // NP)
        pieces.append([
            pltpu.make_async_copy(k_hbm.at[ts, :], kin.at[ts, :], sems.at[7 + 3 * q]),
            pltpu.make_async_copy(v_hbm.at[ts, :], vin.at[ts, :], sems.at[8 + 3 * q]),
            pltpu.make_async_copy(sk_hbm.at[:, ts], skv.at[:, ts], sems.at[9 + 3 * q])])
        for c in pieces[-1]:
            c.start()
    for i in (1, 0, 2):
        cps[i].start()
    qscale = (DH ** -0.5) * math.log2(math.e)

    def proj(r0, xt):
        xn = _ln(xt).astype(BF16)
        kk[pl.ds(r0, TT), :] = jnp.dot(xn, w[:, D:2 * D], preferred_element_type=F32).astype(BF16)
        qT[:, pl.ds(r0, TT)] = (lax.dot_general(wqT[...], xn, NT, preferred_element_type=F32)
                                * qscale).astype(BF16)
        vT[:, pl.ds(r0, TT)] = lax.dot_general(wvT[...], xn, NT, preferred_element_type=F32).astype(BF16)

    sh = sh_ref[...]
    dd = sd_ref[...].astype(F32)
    fw = fw_ref[...]

    def fwd(j, prev):
        r0 = pl.multiple_of(j * L, L)
        kc = kin[pl.ds(r0, L), :].astype(F32)
        kx = jnp.concatenate([prev, kc], 0)
        ks = kc * sh[0:1]
        for d in range(1, 4):
            ks = ks + kx[8 - d:8 - d + L] * sh[d:d + 1]
        kv = ks * vin[pl.ds(r0, L), :].astype(F32)
        y[pl.ds(r0, L), :] = kv * dd
        uf[j] = jnp.dot(fw, kv.astype(BF16), preferred_element_type=F32)
        kf[j] = lax.dot_general(fw, skv[:, pl.ds(r0, L)], NT, preferred_element_type=F32)
        return kc[L - 8:]
    prev = jnp.zeros((8, D), F32)
    for q in range(NP):
        for c in pieces[q]:
            c.wait()
        prev = lax.fori_loop(q * NL // NP, (q + 1) * NL // NP, fwd, prev)

    def prod(b, c):
        ls = pl.ds(pl.multiple_of((b >> 4) * 128, 128), 128)
        HN = NL

        def part(salt, i0, j0, first):
            f0 = pl.multiple_of(((b + 16 * salt) & 15) * 8, 8)
            fr = pl.ds(f0, 8)
            fi = pl.ds(pl.multiple_of(f0 + L, 8), 8)
            ur = [uf[j0 + j, fr, ls] for j in range(HN)]
            ui = [uf[j0 + j, fi, ls] for j in range(HN)]
            for i in range(i0 + HN - 1, i0 - 1, -1):
                ar = ai = None
                if not first:
                    ar, ai = uf[i, fr, ls], uf[i, fi, ls]
                for j in range(min(HN, i - j0 + 1)):
                    kr = kf[i - j0 - j, fr, ls]
                    ki = kf[i - j0 - j, fi, ls]
                    pr = kr * ur[j] - ki * ui[j]
                    pi = kr * ui[j] + ki * ur[j]
                    ar = pr if ar is None else ar + pr
                    ai = pi if ai is None else ai + pi
                uf[i, fr, ls] = ar
                uf[i, fi, ls] = ai
        part(0, 0, 0, True)
        return c
    lax.fori_loop(0, (L // 8) * (D // 128), prod, 0)
    gi = gi_ref[...]

    def inv(i, hi):
        r0 = pl.multiple_of(i * L, L)
        r = jnp.dot(gi, uf[i].astype(BF16), preferred_element_type=F32)
        y[pl.ds(r0, L), :] = y[pl.ds(r0, L), :] + (r[:L] + hi)
        return r[L:]
    lax.fori_loop(0, NL, inv, jnp.zeros((L, D), F32))

    cps[1].wait()

    def tr_body(i, c):
        c0 = pl.multiple_of(i * 128, 128)
        wqT[pl.ds(c0, 128), :] = w[:, pl.ds(c0, 128)].T
        wvT[pl.ds(c0, 128), :] = w[:, pl.ds(pl.multiple_of(2 * D + c0, 128), 128)].T
        return c
    lax.fori_loop(0, D // 128, tr_body, 0)
    cps[0].wait()

    def proj1(t, c):
        r0 = pl.multiple_of(t * TT, TT)
        xt = xin[pl.ds(r0, TT), :].astype(F32)
        xres[pl.ds(r0, TT), :] = xt
        proj(r0, xt)
        return c
    lax.fori_loop(0, S // TT, proj1, 0)

    cps[2].wait()

    row = lax.broadcasted_iota(jnp.int32, (128, TQ), 0)
    nit = H * NQ

    def qk_setup(it):
        h = it >> LNQ
        qt = it & (NQ - 1)
        g = h >> 2
        hh = h & 3
        q = qT[pl.ds(pl.multiple_of(g * 128, 128), 128), pl.ds(pl.multiple_of(qt * TQ, TQ), TQ)]
        qm = jnp.where((row >> 5) == hh, q.astype(F32), 0.0).astype(BF16)
        return g, qm

    def qk_chunk(g, qm, kc, sref):
        kt = kk[pl.ds(kc * KC, KC), pl.ds(pl.multiple_of(g * 128, 128), 128)]
        s = jnp.dot(kt, qm, preferred_element_type=F32)
        sref[pl.ds(kc * KC, KC), :] = s
        return jnp.max(s.reshape(KC // 8, 8, TQ), axis=0)

    def step(it, cur, nxt, mprev8):
        mprev = jnp.max(mprev8, axis=0, keepdims=True)
        h = it >> LNQ
        qt = it & (NQ - 1)
        g, qm = qk_setup(jnp.minimum(it + 1, nit - 1))
        m = acc = l = None
        for kq in range(S // KC + LEAD):
            if kq < S // KC:
                mc = qk_chunk(g, qm, kq, nxt)
                m = mc if m is None else jnp.maximum(m, mc)
            kc = kq - LEAD
            if kc < 0:
                continue
            p = jnp.exp2(cur[pl.ds(kc * KC, KC), :] - mprev)
            lc = jnp.sum(p.reshape(KC // 8, 8, TQ), axis=0)
            l = lc if l is None else l + lc
            vt = vT[pl.ds(pl.multiple_of(h * DH, DH), DH), pl.ds(kc * KC, KC)]
            a = jnp.dot(vt, p.astype(BF16), preferred_element_type=F32)
            acc = a if acc is None else acc + a
        o = acc * (1.0 / jnp.sum(l, axis=0, keepdims=True))
        oT[pl.ds(pl.multiple_of(h * DH, DH), DH), pl.ds(pl.multiple_of(qt * TQ, TQ), TQ)] = o.astype(BF16)
        return m

    def attention():
        g, qm = qk_setup(0)
        m = None
        for kc in range(S // KC):
            mc = qk_chunk(g, qm, kc, sa)
            m = mc if m is None else jnp.maximum(m, mc)

        def body(i2, m):
            for u in range(0, UN, 2):
                m = step(UN * i2 + u, sa, sb, m)
                m = step(UN * i2 + u + 1, sb, sa, m)
            return m
        lax.fori_loop(0, nit // UN, body, m)

    def post(r0):
        rs = pl.ds(r0, TT)
        x1 = xres[rs, :] + lax.dot_general(oT[:, rs], wo[...], TN, preferred_element_type=F32)
        return x1 + _ln(x1) * y[rs, :]

    def layer(li, c):
        attention()

        @pl.when(li == 0)
        def _():
            def mid(t, c2):
                r0 = pl.multiple_of(t * TT, TT)
                x2 = post(r0)
                xres[pl.ds(r0, TT), :] = x2
                proj(r0, x2)
                return c2
            lax.fori_loop(0, S // TT, mid, 0)
        return c
    lax.fori_loop(0, 2, layer, 0)

    def out_copy(t):
        r0 = pl.multiple_of(t * TT, TT)
        return pltpu.make_async_copy(xin.at[pl.ds(r0, TT), :], out_hbm.at[pl.ds(r0, TT), :], sems.at[6])

    def fin(t, c):
        r0 = pl.multiple_of(t * TT, TT)
        xin[pl.ds(r0, TT), :] = post(r0).astype(BF16)
        out_copy(t).start()
        return c
    lax.fori_loop(0, S // TT, fin, 0)
    pltpu.make_async_copy(xin, out_hbm, sems.at[6]).wait()


@jax.jit
def pallas_interleave_layers__softmax_full_mha__ssm_conv_h3__prompt_kernel(
    A_x, A_wqkv, A_wo, B_q, B_k, B_v, B_shift_k, B_ssm_k, B_ssm_D,
):
    fwd, inv = _dft_consts()
    any_spec = pl.BlockSpec(memory_space=pl.ANY)
    vmem_spec = pl.BlockSpec(memory_space=pltpu.VMEM)
    vm = pltpu.VMEM
    out = pl.pallas_call(
        _kernel,
        out_shape=jax.ShapeDtypeStruct((S, D), BF16),
        in_specs=[any_spec] * 5 + [vmem_spec, any_spec, vmem_spec, vmem_spec, vmem_spec],
        out_specs=any_spec,
        scratch_shapes=[
            vm((S, D), BF16), vm((S, D), F32), vm((D, 3 * D), BF16), vm((D, D), BF16),
            vm((D, D), BF16), vm((D, D), BF16),
            vm((D, S), BF16), vm((S, D), BF16), vm((D, S), BF16), vm((D, S), BF16),
            vm((S, TQ), F32), vm((S, TQ), F32), vm((S, D), F32),
            vm((S, D), BF16), vm((S, D), BF16), vm((D, S), BF16),
            vm((NL, 2 * L, D), F32), vm((NL, 2 * L, D), F32),
            pltpu.SemaphoreType.DMA((7 + 3 * NP,)),
        ],
        compiler_params=pltpu.CompilerParams(vmem_limit_bytes=120 * 1024 * 1024),
    )(A_x.reshape(S, D), A_wqkv, A_wo, B_k.reshape(S, D), B_v.reshape(S, D),
      B_shift_k.T.astype(F32), B_ssm_k, B_ssm_D.reshape(1, D),
      jnp.asarray(fwd, BF16), jnp.asarray(inv, BF16))
    return out.reshape(A_x.shape)
```
